```python
import jax
import jax.numpy as jnp

def _softmax(x, axis=-1):
    return jax.nn.softmax(x, axis=axis)

def _gelu(x):
    return jax.nn.gelu(x, approximate=True)

def _silu(x):
    return jax.nn.silu(x)

def _sigmoid(x):
    return jax.nn.sigmoid(x)

def _layernorm(x, axis=-1, eps=1e-05):
    m = jnp.mean(x, axis=axis, keepdims=True)
    v = jnp.var(x, axis=axis, keepdims=True)
    return (x - m) / jnp.sqrt(v + eps)

def _scatter_add(tgt, idx, src, axis=0):
    return tgt.at[idx].add(src)

def _segment_sum(src, seg, n):
    return jax.ops.segment_sum(src, seg, n)

class _Rng:

    def __init__(self, key):
        self._k = key

    def _next(self):
        self._k, sub = jax.random.split(self._k)
        return sub

    def normal(self, shape):
        return jax.random.normal(self._next(), shape, dtype=jnp.bfloat16)

    def randint(self, lo, hi, shape):
        return jax.random.randint(self._next(), shape, lo, hi, dtype=jnp.int32)

    def uniform(self, shape, lo=0.0, hi=1.0):
        return jax.random.uniform(self._next(), shape, jnp.bfloat16, lo, hi)

    def permutation(self, n):
        return jax.random.permutation(self._next(), n)
kernel_name = 'adaLN_cond__sliding_block_cached__glu_gated_swiglu__decode'

def setup_inputs():
    _rng = _Rng(jax.random.key(int.from_bytes(__import__("os").urandom(4), "little")))
    _w = lambda a: (lambda t: t.astype(jnp.bfloat16) if jnp.issubdtype(t.dtype, jnp.floating) else t)(jnp.asarray(a))

    def _A_setup():
        B, Sq, D = (2, 1, 512)
        Hq, Hkv, Sk, Dh = (32, 32, 16384, 128)
        assert Hq % Hkv == 0, (Hq, Hkv)
        return {'x': _w((lambda *s: _rng.normal(s) * 0.05)(B, Sq, D)), 'k_cache': _w((lambda *s: _rng.normal(s) * 0.05)(B, Hkv, Sk, Dh)), 'v_cache': _w((lambda *s: _rng.normal(s) * 0.05)(B, Hkv, Sk, Dh)), 'wq': _w((lambda *s: _rng.normal(s) * 0.05)(D, Hq * Dh) * D ** (-0.5)), 'wo': _w((lambda *s: _rng.normal(s) * 0.05)(Hq * Dh, D) * (Hq * Dh) ** (-0.5))}
    _A_in = _A_setup()

    def _B_setup():
        B, S, D, F = (2, 1, 512, 1376)
        return {'x': _w((lambda *s: _rng.normal(s) * 0.05)(B, S, D)), 'w1': _w((lambda *s: _rng.normal(s) * 0.05)(D, F) * (2.0 / D) ** 0.5), 'w3': _w((lambda *s: _rng.normal(s) * 0.05)(D, F) * (2.0 / D) ** 0.5), 'w2': _w((lambda *s: _rng.normal(s) * 0.05)(F, D) * (2.0 / F) ** 0.5)}
    _B_in = _B_setup()
    return {'A_x': _A_in['x'], 'A_k_cache': _A_in['k_cache'], 'A_v_cache': _A_in['v_cache'], 'A_wq': _A_in['wq'], 'A_wo': _A_in['wo'], 'B_x': _B_in['x'], 'B_w1': _B_in['w1'], 'B_w3': _B_in['w3'], 'B_w2': _B_in['w2'], 'c': _w((lambda *s: _rng.normal(s) * 0.05)(2, 512)), 'w_mod': _w((lambda *s: _rng.normal(s) * 0.05)(512, 6 * 512) * 512 ** (-0.5))}

def reference(A_x, A_k_cache, A_v_cache, A_wq, A_wo, B_x, B_w1, B_w3, B_w2, c, w_mod):

    def _A_ref(x, k_cache, v_cache, wq, wo):
        B, Sq, D = x.shape
        Hq, Dh = (32, 128)
        Hkv, Sk = (k_cache.shape[1], k_cache.shape[2])
        W = min(4096, max(256, Sk // 4))
        rep = Hq // Hkv
        q = (lambda x, *d: x.transpose(*d))((x @ wq).reshape(B, Sq, Hq, Dh), 0, 2, 1, 3)
        k = jnp.repeat(k_cache[:, :, Sk - W:, :], rep, axis=1)
        v = jnp.repeat(v_cache[:, :, Sk - W:, :], rep, axis=1)
        scores = jnp.einsum('bhqd,bhkd->bhqk', q, k) * Dh ** (-0.5)
        p = _softmax(scores, axis=-1)
        o = jnp.einsum('bhqk,bhkd->bhqd', p, v)
        return (lambda x, *d: x.transpose(*d))(o, 0, 2, 1, 3).reshape(B, Sq, Hq * Dh) @ wo

    def _B_ref(x, w1, w3, w2):
        gate = jnp.einsum('bsd,df->bsf', x, w1)
        up = jnp.einsum('bsd,df->bsf', x, w3)
        h = _silu(gate) * up
        out = jnp.einsum('bsf,fd->bsd', h, w2)
        return out
    x = A_x
    mod = (_silu(c) @ w_mod).reshape(c.shape[0], 6, 1, -1)
    sa, ca, ga, sb, cb, gb = (mod[:, 0].copy(), mod[:, 1].copy(), mod[:, 2].copy(), mod[:, 3].copy(), mod[:, 4].copy(), mod[:, 5].copy())
    h = _layernorm(x, axis=-1) * (1 + ca) + sa
    x = x + ga * _A_ref(h, A_k_cache, A_v_cache, A_wq, A_wo)
    h = _layernorm(x, axis=-1) * (1 + cb) + sb
    x = x + gb * _B_ref(h, B_w1, B_w3, B_w2)
    return x
```

```python
import functools
import jax
import jax.numpy as jnp
from jax import lax
import jax.experimental.pallas as pl
import jax.experimental.pallas.tpu as pltpu

F32 = jnp.float32
BF16 = jnp.bfloat16
NT = (((1,), (1,)), ((), ()))


def _silu(x):
    return x * (1.0 / (1.0 + jnp.exp(-x)))


def _layernorm(x, eps=1e-5):
    m = jnp.mean(x, axis=-1, keepdims=True)
    d = x - m
    v = jnp.mean(d * d, axis=-1, keepdims=True)
    return d / jnp.sqrt(v + eps)


def make(name="k1", depth=8, two_prio=True):
    B, H, S, Dh, D, F = 2, 32, 16384, 128, 512, 1376
    W = min(4096, max(256, S // 4))
    NBH = B * H
    W2_CHUNKS = [(0, 512), (512, 512), (1024, 256), (1280, 96)]

    def kern(x_hbm, k_hbm, v_hbm, wq_hbm, wo_hbm, w1_hbm, w3_hbm, w2_hbm, c_hbm, wm_hbm, o_hbm,
             kbuf, vbuf, ksem, vsem, xb, cb_, wmb, wqb, wob, w1b, w3b, w2b, wsem, w2sem, qs, os_, ob, osem):
        p1 = 1 if two_prio else 0
        cp_c = pltpu.make_async_copy(c_hbm, cb_, wsem.at[0])
        cp_x = pltpu.make_async_copy(x_hbm, xb, wsem.at[1])
        cp_wm = pltpu.make_async_copy(wm_hbm, wmb, wsem.at[2])
        cp_wq = pltpu.make_async_copy(wq_hbm, wqb, wsem.at[3])
        cp_wo = pltpu.make_async_copy(wo_hbm, wob, wsem.at[4])
        cp_w1 = pltpu.make_async_copy(w1_hbm, w1b, wsem.at[5])
        cp_w3 = pltpu.make_async_copy(w3_hbm, w3b, wsem.at[6])
        cp_w2 = [pltpu.make_async_copy(w2_hbm.at[pl.ds(s, n), :], w2b.at[pl.ds(s, n), :], w2sem.at[i])
                 for i, (s, n) in enumerate(W2_CHUNKS)]

        def kcopy(i, slot):
            return pltpu.make_async_copy(k_hbm.at[i % B, i // B, pl.ds(S - W, W), :], kbuf.at[slot], ksem.at[slot])

        def vcopy(i, slot):
            return pltpu.make_async_copy(v_hbm.at[i % B, i // B, pl.ds(S - W, W), :], vbuf.at[slot], vsem.at[slot])

        cp_wm.start(priority=0)
        cp_wq.start(priority=p1)
        cp_c.start(priority=0)
        cp_x.start(priority=0)
        cp_wo.start(priority=0)
        for i in range(depth):
            kcopy(i, i).start(priority=p1)
            vcopy(i, i).start(priority=0)

        cp_c.wait()
        cp_wm.wait()
        cp_x.wait()
        sc = _silu(cb_[...].astype(F32)).astype(BF16)
        mod = jnp.dot(sc, wmb[...], preferred_element_type=F32)
        sa, ca, ga, sb, cb, gb = [mod[:, j * D:(j + 1) * D] for j in range(6)]
        x = xb[...].astype(F32)
        h = _layernorm(x) * (1.0 + ca) + sa
        cp_wq.wait()
        q = jnp.dot(h.astype(BF16), wqb[...], preferred_element_type=F32)
        for hh in range(H):
            qs[hh] = q[:, hh * Dh:(hh + 1) * Dh]
        os_[...] = jnp.zeros_like(os_)

        scale = Dh ** -0.5
        row = lax.broadcasted_iota(jnp.int32, (B, Dh), 0)

        def body(i, _):
            slot = i % depth
            hh = i // B
            b = i % B
            kcopy(i, slot).wait()
            s = lax.dot_general(qs[hh].astype(BF16), kbuf[slot], NT, preferred_element_type=F32) * scale

            @pl.when(i + depth < NBH)
            def _():
                kcopy(i + depth, slot).start(priority=p1)

            m = jnp.max(s, axis=-1, keepdims=True)
            p = jnp.exp(s - m)
            l = jnp.sum(p, axis=-1, keepdims=True)
            vcopy(i, slot).wait()
            o = jnp.dot(p.astype(BF16), vbuf[slot], preferred_element_type=F32) / l
            os_[hh] = jnp.where(row == b, o, os_[hh])

            @pl.when(i + depth < NBH)
            def _():
                vcopy(i + depth, slot).start(priority=0)

            @pl.when(i + depth == NBH - 1)
            def _():
                cp_w1.start(priority=p1)
                cp_w3.start(priority=0)
                for j, cp in enumerate(cp_w2):
                    cp.start(priority=p1 if j % 2 == 0 else 0)
            return 0

        lax.fori_loop(0, NBH, body, 0)

        cp_wo.wait()
        o_all = jnp.concatenate([os_[hh] for hh in range(H)], axis=-1)
        attn = jnp.dot(o_all.astype(BF16), wob[...], preferred_element_type=F32)
        x1 = x + ga * attn
        h2 = (_layernorm(x1) * (1.0 + cb) + sb).astype(BF16)
        cp_w1.wait()
        gate = lax.dot_general(h2, w1b[...], NT, preferred_element_type=F32)
        cp_w3.wait()
        up = lax.dot_general(h2, w3b[...], NT, preferred_element_type=F32)
        act = (_silu(gate) * up).astype(BF16)
        acc = jnp.zeros((B, D), F32)
        for j, (s_, n) in enumerate(W2_CHUNKS):
            cp_w2[j].wait()
            acc = acc + jnp.dot(act[:, s_:s_ + n], w2b[pl.ds(s_, n), :], preferred_element_type=F32)
        ob[...] = (x1 + gb * acc).astype(BF16)
        cp_o = pltpu.make_async_copy(ob, o_hbm, osem)
        cp_o.start()
        cp_o.wait()

    def fn(A_x, A_k_cache, A_v_cache, A_wq, A_wo, B_x, B_w1, B_w3, B_w2, c, w_mod):
        any_ = pl.BlockSpec(memory_space=pl.ANY)
        out = pl.pallas_call(
            kern,
            out_shape=jax.ShapeDtypeStruct((B, D), BF16),
            in_specs=[any_] * 10,
            out_specs=any_,
            scratch_shapes=[
                pltpu.VMEM((depth, W, Dh), BF16), pltpu.VMEM((depth, W, Dh), BF16),
                pltpu.SemaphoreType.DMA((depth,)), pltpu.SemaphoreType.DMA((depth,)),
                pltpu.VMEM((B, D), BF16), pltpu.VMEM((B, D), BF16),
                pltpu.VMEM((D, 6 * D), BF16), pltpu.VMEM((D, H * Dh), BF16), pltpu.VMEM((H * Dh, D), BF16),
                pltpu.VMEM((F, D), BF16), pltpu.VMEM((F, D), BF16), pltpu.VMEM((F, D), BF16),
                pltpu.SemaphoreType.DMA((7,)), pltpu.SemaphoreType.DMA((len(W2_CHUNKS),)),
                pltpu.VMEM((H, B, Dh), F32), pltpu.VMEM((H, B, Dh), F32),
                pltpu.VMEM((B, D), BF16), pltpu.SemaphoreType.DMA(()),
            ],
            compiler_params=pltpu.CompilerParams(vmem_limit_bytes=100 * 1024 * 1024),
            name=name,
        )(A_x.reshape(B, D), A_k_cache, A_v_cache, A_wq, A_wo, B_w1.T, B_w3.T, B_w2, c, w_mod)
        return out.reshape(B, 1, D)
    return fn


_kernel = make("adaln_decode", depth=4, two_prio=True)


@jax.jit
def pallas_adaLN_cond__sliding_block_cached__glu_gated_swiglu__decode_kernel(
    A_x, A_k_cache, A_v_cache, A_wq, A_wo, B_x, B_w1, B_w3, B_w2, c, w_mod):
    return _kernel(A_x, A_k_cache, A_v_cache, A_wq, A_wo, B_x, B_w1, B_w3, B_w2, c, w_mod)
```

```python
import contextlib
import jax
import jax.numpy as jnp
from jax import lax
import jax.experimental.pallas as pl
import jax.experimental.pallas.tpu as pltpu

F32 = jnp.float32
BF16 = jnp.bfloat16
NT = (((1,), (1,)), ((), ()))


def _silu(x):
    return x * (1.0 / (1.0 + jnp.exp(-x)))


def _layernorm(x, eps=1e-5):
    m = jnp.mean(x, axis=-1, keepdims=True)
    d = x - m
    v = jnp.mean(d * d, axis=-1, keepdims=True)
    return d / jnp.sqrt(v + eps)


def make(name="k3", depth=3, rows=128, nseg=2, wrows=16, prows0=128, prows1=128, scopes=False, nochk=True,
         w2_chunks=((0, 1152), (1152, 224)), two_stream_w=True, vshift=576, lastp=(1,)):
    B, H, S, Dh, D, F = 2, 32, 16384, 128, 512, 1376
    W = min(4096, max(256, S // 4))
    NBH = B * H
    scope = (lambda n: jax.named_scope(n)) if scopes else (lambda n: contextlib.nullcontext())
    assert depth == 3

    def kern(x_hbm, k_hbm, v_hbm, wq_hbm, wo_hbm, w1_hbm, w3_hbm, w2_hbm, c_hbm, wm_hbm, o_hbm,
             kv, xb, cb_, wmb, wqb, wob, w1b, w3b, w2b, qs, os_, ob, sem):

        def pieces(src, dst, r0, nr, prows):
            piece = prows * Dh
            cdim = src.shape[1]
            lanes = min(cdim, piece // wrows)
            step = max(wrows, piece // lanes)
            out = []
            for st in range(r0, r0 + nr, step):
                sz = min(step, r0 + nr - st)
                for cs in range(0, cdim, lanes):
                    n = min(lanes, cdim - cs)
                    out.append((src.at[pl.ds(st, sz), pl.ds(cs, n)], dst.at[pl.ds(st, sz), pl.ds(cs, n)]))
            return out

        def start_all(ps, s):
            n = len(ps)
            if two_stream_w:
                half = (n + 1) // 2
                order_ = []
                for j in range(half):
                    order_.append(j)
                    if half + j < n:
                        order_.append(half + j)
            else:
                order_ = range(n)
            for j, idx in enumerate(order_):
                a, b_ = ps[idx]
                pltpu.make_async_copy(a, b_, s).start(priority=j % 2)

        def start_w(src, dst, s, prows, r0=0, nr=None):
            start_all(pieces(src, dst, r0, src.shape[0] if nr is None else nr, prows), s)

        def wait_buf(buf, s):
            pltpu.make_async_copy(buf, buf, s).wait()

        def start_head(i, slot):
            b = i % B
            hh = i // B
            seg = W // nseg
            for st in range(0, seg, rows):
                for j in range(nseg):
                    r = j * seg + st
                    pltpu.make_async_copy(k_hbm.at[b, hh, pl.ds(S - W + r, rows), :], kv.at[slot, 0, pl.ds(r, rows), :], sem.at[slot]).start(priority=0)
                    rv = (st + vshift) % seg
                    for a_, n_ in ([(rv, rows)] if rv + rows <= seg else [(rv, seg - rv), (0, rows - (seg - rv))]):
                        a_ += j * seg
                        pltpu.make_async_copy(v_hbm.at[b, hh, pl.ds(S - W + a_, n_), :], kv.at[slot, 1, pl.ds(a_, n_), :], sem.at[slot]).start(priority=1)

        ws = sem.at[depth]
        cp_c = pltpu.make_async_copy(c_hbm, cb_, ws)
        cp_x = pltpu.make_async_copy(x_hbm, xb, ws)
        start_w(wm_hbm, wmb, ws, prows0)
        cp_c.start(priority=0)
        cp_x.start(priority=1)
        start_w(wq_hbm, wqb, sem.at[depth - 1], prows0)
        with scope("W_wm"):
            cp_c.wait()
            cp_x.wait()
            wait_buf(wmb, ws)
        sc = _silu(cb_[...].astype(F32)).astype(BF16)
        mod = jnp.dot(sc, wmb[...], preferred_element_type=F32)
        sa, ca, ga, sb, cb, gb = [mod[:, j * D:(j + 1) * D] for j in range(6)]
        x = xb[...].astype(F32)
        h = (_layernorm(x) * (1.0 + ca) + sa).astype(BF16)
        for i in range(depth - 1):
            start_head(i, i)
        with scope("W_wq"):
            wait_buf(wqb, sem.at[depth - 1])
        q = jnp.dot(h, wqb[...], preferred_element_type=F32)
        for hh in range(H):
            qs[hh] = q[:, hh * Dh:(hh + 1) * Dh]
        os_[...] = jnp.zeros_like(os_)
        start_head(depth - 1, depth - 1)

        scale = Dh ** -0.5
        row = lax.broadcasted_iota(jnp.int32, (B, Dh), 0)

        def attend(i):
            slot = i % depth
            hh = i // B
            b = i % B
            with scope("W_kv"):
                wait_buf(kv.at[slot], sem.at[slot])
            s = lax.dot_general(qs[hh].astype(BF16), kv[slot, 0], NT, preferred_element_type=F32) * scale
            m = jnp.max(s, axis=-1, keepdims=True)
            p = jnp.exp(s - m)
            l = jnp.sum(p, axis=-1, keepdims=True)
            o = jnp.dot(p.astype(BF16), kv[slot, 1], preferred_element_type=F32) / l
            os_[hh] = jnp.where(row == b, o, os_[hh])

        def body(i, _):
            attend(i)
            start_head(i + depth, i % depth)
            return 0

        lax.fori_loop(0, NBH - depth, body, 0)
        sl = [sem.at[(NBH - depth + j) % depth] for j in range(depth)]

        def start_last():
            p3 = [(a_, b_, sl[1]) for a_, b_ in pieces(w3_hbm, w3b, 0, F, prows1)]
            p2 = [(a_, b_, sl[2]) for a_, b_ in pieces(w2_hbm, w2b, *w2_chunks[0], prows1)]
            for j in range(max(len(p3), len(p2))):
                if j < len(p3):
                    pltpu.make_async_copy(*p3[j]).start(priority=0)
                if j < len(p2):
                    pltpu.make_async_copy(*p2[j]).start(priority=1)

        tail = [lambda: start_w(wo_hbm, wob, ws, prows1),
                lambda: start_w(w1_hbm, w1b, sl[0], prows1),
                start_last]

        def body2(i, _):
            attend(i)
            for j in range(depth):
                @pl.when(i == NBH - depth + j)
                def _():
                    tail[j]()
            return 0
        lax.fori_loop(NBH - depth, NBH, body2, 0)

        with scope("W_wo"):
            wait_buf(wob, ws)
        for j, (a_, b_) in enumerate(pieces(w2_hbm, w2b, *w2_chunks[1], prows1)):
            pltpu.make_async_copy(a_, b_, ws).start(priority=lastp[j % len(lastp)])
        o_all = jnp.concatenate([os_[hh] for hh in range(H)], axis=-1)
        attn = jnp.dot(o_all.astype(BF16), wob[...], preferred_element_type=F32)
        x1 = x + ga * attn
        h2 = (_layernorm(x1) * (1.0 + cb) + sb).astype(BF16)
        with scope("W_w1"):
            wait_buf(w1b, sl[0])
        gate = lax.dot_general(h2, w1b[...], NT, preferred_element_type=F32)
        gs = _silu(gate)
        with scope("W_w3"):
            wait_buf(w3b, sl[1])
        up = lax.dot_general(h2, w3b[...], NT, preferred_element_type=F32)
        act = (gs * up).astype(BF16)
        acc = jnp.zeros((B, D), F32)
        for (s_, n), sm in zip(w2_chunks, (sl[2], ws)):
            with scope("W_w2"):
                wait_buf(w2b.at[pl.ds(s_, n), :], sm)
            acc = acc + jnp.dot(act[:, s_:s_ + n], w2b[pl.ds(s_, n), :], preferred_element_type=F32)
        ob[...] = (x1 + gb * acc).astype(BF16)
        cp_o = pltpu.make_async_copy(ob, o_hbm, sl[1])
        cp_o.start()
        with scope("W_o"):
            cp_o.wait()

    def fn(A_x, A_k_cache, A_v_cache, A_wq, A_wo, B_x, B_w1, B_w3, B_w2, c, w_mod):
        any_ = pl.BlockSpec(memory_space=pl.ANY)
        out = pl.pallas_call(
            kern,
            out_shape=jax.ShapeDtypeStruct((B, D), BF16),
            in_specs=[any_] * 10,
            out_specs=any_,
            scratch_shapes=[
                pltpu.VMEM((depth, 2, W, Dh), BF16),
                pltpu.VMEM((B, D), BF16), pltpu.VMEM((B, D), BF16),
                pltpu.VMEM((D, 6 * D), BF16), pltpu.VMEM((D, H * Dh), BF16), pltpu.VMEM((H * Dh, D), BF16),
                pltpu.VMEM((F, D), BF16), pltpu.VMEM((F, D), BF16), pltpu.VMEM((F, D), BF16),
                pltpu.VMEM((H, B, Dh), F32), pltpu.VMEM((H, B, Dh), F32),
                pltpu.VMEM((B, D), BF16), pltpu.SemaphoreType.DMA((depth + 1,)),
            ],
            compiler_params=pltpu.CompilerParams(vmem_limit_bytes=100 * 1024 * 1024, disable_bounds_checks=nochk, disable_semaphore_checks=nochk),
            name=name,
        )(A_x.reshape(B, D), A_k_cache, A_v_cache, A_wq, A_wo, B_w1.T, B_w3.T, B_w2, c, w_mod)
        return out.reshape(B, 1, D)
    return fn


_kernel = make("adaln_decode", wrows=8, w2_chunks=((0,1024),(1024,352)))


@jax.jit
def pallas_adaLN_cond__sliding_block_cached__glu_gated_swiglu__decode_kernel(
    A_x, A_k_cache, A_v_cache, A_wq, A_wo, B_x, B_w1, B_w3, B_w2, c, w_mod):
    return _kernel(A_x, A_k_cache, A_v_cache, A_wq, A_wo, B_x, B_w1, B_w3, B_w2, c, w_mod)
```

```python
import contextlib
import jax
import jax.numpy as jnp
from jax import lax
import jax.experimental.pallas as pl
import jax.experimental.pallas.tpu as pltpu

F32 = jnp.float32
BF16 = jnp.bfloat16
NT = (((1,), (1,)), ((), ()))


def _silu(x):
    return x * (1.0 / (1.0 + jnp.exp(-x)))


def _layernorm(x, eps=1e-5):
    m = jnp.mean(x, axis=-1, keepdims=True)
    d = x - m
    v = jnp.mean(d * d, axis=-1, keepdims=True)
    return d / jnp.sqrt(v + eps)


def make(name="k3", depth=3, rows=128, nseg=2, wrows=8, prows0=128, prows1=128, scopes=False, nochk=True,
         w2_chunks=((0, 1024), (1024, 352)), nsw=2, wshift=0, vshift=576, lastp=(1,)):
    B, H, S, Dh, D, F = 2, 32, 16384, 128, 512, 1376
    W = min(4096, max(256, S // 4))
    NBH = B * H
    scope = (lambda n: jax.named_scope(n)) if scopes else (lambda n: contextlib.nullcontext())
    assert depth == 3

    def kern(x_hbm, k_hbm, v_hbm, wq_hbm, wo_hbm, w1_hbm, w3_hbm, w2_hbm, c_hbm, wm_hbm, o_hbm,
             kv, xb, cb_, wmb, wqb, wob, w1b, w3b, w2b, qs, os_, accb, ob, sem):

        def pieces(src, dst, r0, nr, prows):
            piece = prows * Dh
            cdim = src.shape[1]
            lanes = min(cdim, piece // wrows)
            step = max(wrows, piece // lanes)
            out = []
            for st in range(r0, r0 + nr, step):
                sz = min(step, r0 + nr - st)
                for cs in range(0, cdim, lanes):
                    n = min(lanes, cdim - cs)
                    out.append((src.at[pl.ds(st, sz), pl.ds(cs, n)], dst.at[pl.ds(st, sz), pl.ds(cs, n)]))
            return out

        def start_all(ps, s):
            n = len(ps)
            seg = -(-n // nsw)
            order_ = []
            for j in range(seg):
                for t in range(nsw):
                    ln = min(seg, n - t * seg)
                    if j < ln:
                        order_.append(t * seg + (j + (wshift if t % 2 else 0)) % ln)
            assert sorted(order_) == list(range(n))
            for j, idx in enumerate(order_):
                a, b_ = ps[idx]
                pltpu.make_async_copy(a, b_, s).start(priority=j % 2)

        def start_w(src, dst, s, prows, r0=0, nr=None):
            start_all(pieces(src, dst, r0, src.shape[0] if nr is None else nr, prows), s)

        def wait_buf(buf, s):
            pltpu.make_async_copy(buf, buf, s).wait()

        def start_head(i, slot):
            b = i % B
            hh = i // B
            seg = W // nseg
            for st in range(0, seg, rows):
                for j in range(nseg):
                    r = j * seg + st
                    pltpu.make_async_copy(k_hbm.at[b, hh, pl.ds(S - W + r, rows), :], kv.at[slot, 0, pl.ds(r, rows), :], sem.at[slot]).start(priority=0)
                    rv = (st + vshift) % seg
                    for a_, n_ in ([(rv, rows)] if rv + rows <= seg else [(rv, seg - rv), (0, rows - (seg - rv))]):
                        a_ += j * seg
                        pltpu.make_async_copy(v_hbm.at[b, hh, pl.ds(S - W + a_, n_), :], kv.at[slot, 1, pl.ds(a_, n_), :], sem.at[slot]).start(priority=1)

        ws = sem.at[depth]
        cp_c = pltpu.make_async_copy(c_hbm, cb_, ws)
        cp_x = pltpu.make_async_copy(x_hbm, xb, ws)
        start_w(wm_hbm, wmb, ws, prows0)
        cp_c.start(priority=0)
        cp_x.start(priority=1)
        start_w(wq_hbm, wqb, sem.at[depth - 1], prows0)
        with scope("W_wm"):
            cp_c.wait()
            cp_x.wait()
            wait_buf(wmb, ws)
        sc = _silu(cb_[...].astype(F32)).astype(BF16)
        mod = jnp.dot(sc, wmb[...], preferred_element_type=F32)
        sa, ca, ga, sb, cb, gb = [mod[:, j * D:(j + 1) * D] for j in range(6)]
        x = xb[...].astype(F32)
        h = (_layernorm(x) * (1.0 + ca) + sa).astype(BF16)
        for i in range(depth - 1):
            start_head(i, i)
        with scope("W_wq"):
            wait_buf(wqb, sem.at[depth - 1])
        q = jnp.dot(h, wqb[...], preferred_element_type=F32)
        for hh in range(H):
            qs[hh] = q[:, hh * Dh:(hh + 1) * Dh]
        os_[...] = jnp.zeros_like(os_)
        start_head(depth - 1, depth - 1)

        scale = Dh ** -0.5
        row = lax.broadcasted_iota(jnp.int32, (B, Dh), 0)

        def attend(i):
            slot = i % depth
            hh = i // B
            b = i % B
            with scope("W_kv"):
                wait_buf(kv.at[slot], sem.at[slot])
            s = lax.dot_general(qs[hh].astype(BF16), kv[slot, 0], NT, preferred_element_type=F32) * scale
            m = jnp.max(s, axis=-1, keepdims=True)
            p = jnp.exp(s - m)
            l = jnp.sum(p, axis=-1, keepdims=True)
            o = jnp.dot(p.astype(BF16), kv[slot, 1], preferred_element_type=F32) / l
            os_[hh] = jnp.where(row == b, o, os_[hh])

        def body(i, _):
            attend(i)
            start_head(i + depth, i % depth)
            return 0

        lax.fori_loop(0, NBH - depth, body, 0)
        sl = [sem.at[(NBH - depth + j) % depth] for j in range(depth)]

        def start_last():
            p3 = [(a_, b_, sl[1]) for a_, b_ in pieces(w3_hbm, w3b, 0, F, prows1)]
            p2 = [(a_, b_, sl[2]) for a_, b_ in pieces(w2_hbm, w2b, *w2_chunks[0], prows1)]
            for j in range(max(len(p3), len(p2))):
                if j < len(p3):
                    pltpu.make_async_copy(*p3[j]).start(priority=0)
                if j < len(p2):
                    pltpu.make_async_copy(*p2[j]).start(priority=1)

        tail = [lambda: start_w(wo_hbm, wob, ws, prows1),
                lambda: start_w(w1_hbm, w1b, sl[0], prows1),
                start_last]

        def body2(i, _):
            attend(i)
            for j in range(depth):
                @pl.when(i == NBH - depth + j)
                def _():
                    tail[j]()
            return 0
        lax.fori_loop(NBH - depth, NBH, body2, 0)

        with scope("W_wo"):
            wait_buf(wob, ws)
        for j, (a_, b_) in enumerate(pieces(w2_hbm, w2b, *w2_chunks[1], prows1)):
            pltpu.make_async_copy(a_, b_, ws).start(priority=lastp[j % len(lastp)])
        o_all = jnp.concatenate([os_[hh] for hh in range(H)], axis=-1)
        attn = jnp.dot(o_all.astype(BF16), wob[...], preferred_element_type=F32)
        x1 = x + ga * attn
        h2 = (_layernorm(x1) * (1.0 + cb) + sb).astype(BF16)
        with scope("W_w1"):
            wait_buf(w1b, sl[0])
        gate = lax.dot_general(h2, w1b[...], NT, preferred_element_type=F32)
        gs = _silu(gate)
        with scope("W_w3"):
            wait_buf(w3b, sl[1])
        up = lax.dot_general(h2, w3b[...], NT, preferred_element_type=F32)
        act = (gs * up).astype(BF16)
        (s0, n0), (s1, n1) = w2_chunks
        with scope("W_w2"):
            wait_buf(w2b.at[pl.ds(s0, n0), :], sl[2])
        accb[...] = x1 + gb * jnp.dot(act[:, s0:s0 + n0], w2b[pl.ds(s0, n0), :], preferred_element_type=F32)
        with scope("W_w2"):
            wait_buf(w2b.at[pl.ds(s1, n1), :], ws)
        ob[...] = (accb[...] + gb * jnp.dot(act[:, s1:s1 + n1], w2b[pl.ds(s1, n1), :], preferred_element_type=F32)).astype(BF16)
        cp_o = pltpu.make_async_copy(ob, o_hbm, sl[1])
        cp_o.start()
        with scope("W_o"):
            cp_o.wait()

    def fn(A_x, A_k_cache, A_v_cache, A_wq, A_wo, B_x, B_w1, B_w3, B_w2, c, w_mod):
        any_ = pl.BlockSpec(memory_space=pl.ANY)
        out = pl.pallas_call(
            kern,
            out_shape=jax.ShapeDtypeStruct((B, D), BF16),
            in_specs=[any_] * 10,
            out_specs=any_,
            scratch_shapes=[
                pltpu.VMEM((depth, 2, W, Dh), BF16),
                pltpu.VMEM((B, D), BF16), pltpu.VMEM((B, D), BF16),
                pltpu.VMEM((D, 6 * D), BF16), pltpu.VMEM((D, H * Dh), BF16), pltpu.VMEM((H * Dh, D), BF16),
                pltpu.VMEM((F, D), BF16), pltpu.VMEM((F, D), BF16), pltpu.VMEM((F, D), BF16),
                pltpu.VMEM((H, B, Dh), F32), pltpu.VMEM((H, B, Dh), F32),
                pltpu.VMEM((B, D), F32), pltpu.VMEM((B, D), BF16), pltpu.SemaphoreType.DMA((depth + 1,)),
            ],
            compiler_params=pltpu.CompilerParams(vmem_limit_bytes=100 * 1024 * 1024, disable_bounds_checks=nochk, disable_semaphore_checks=nochk),
            name=name,
        )(A_x.reshape(B, D), A_k_cache, A_v_cache, A_wq, A_wo, B_w1.T, B_w3.T, B_w2, c, w_mod)
        return out.reshape(B, 1, D)
    return fn


_kernel = make("adaln_decode", nsw=4, wshift=5, w2_chunks=((0,1024),(1024,352)))


@jax.jit
def pallas_adaLN_cond__sliding_block_cached__glu_gated_swiglu__decode_kernel(
    A_x, A_k_cache, A_v_cache, A_wq, A_wo, B_x, B_w1, B_w3, B_w2, c, w_mod):
    return _kernel(A_x, A_k_cache, A_v_cache, A_wq, A_wo, B_x, B_w1, B_w3, B_w2, c, w_mod)
```

```python
import contextlib
import jax
import jax.numpy as jnp
from jax import lax
import jax.experimental.pallas as pl
import jax.experimental.pallas.tpu as pltpu

F32 = jnp.float32
BF16 = jnp.bfloat16
NT = (((1,), (1,)), ((), ()))


def _silu(x):
    return x * (1.0 / (1.0 + jnp.exp(-x)))


def _layernorm(x, eps=1e-5):
    m = jnp.mean(x, axis=-1, keepdims=True)
    d = x - m
    v = jnp.mean(d * d, axis=-1, keepdims=True)
    return d / jnp.sqrt(v + eps)


def make(name="k3", depth=2, rows=128, kshift=0, e=0, wrows=8, prows0=128, prows1=128, scopes=False, nochk=True,
         w2_chunks=((0, 1024), (1024, 352)), nsw=4, wshift=5, vshift=576, lastp=(1,)):
    B, H, S, Dh, D, F = 2, 32, 16384, 128, 512, 1376
    W = min(4096, max(256, S // 4))
    NBH = B * H
    scope = (lambda n: jax.named_scope(n)) if scopes else (lambda n: contextlib.nullcontext())
    assert depth == 2

    def kern(x_hbm, k_hbm, v_hbm, wq_hbm, wo_hbm, w1_hbm, w3_hbm, w2_hbm, c_hbm, wm_hbm, o_hbm,
             kv, xb, cb_, wmb, wqb, wob, w1b, w3b, w2b, qs, os_, accb, ob, sem):

        def pieces(src, dst, r0, nr, prows):
            piece = prows * Dh
            cdim = src.shape[1]
            lanes = min(cdim, piece // wrows)
            step = max(wrows, piece // lanes)
            out = []
            for st in range(r0, r0 + nr, step):
                sz = min(step, r0 + nr - st)
                for cs in range(0, cdim, lanes):
                    n = min(lanes, cdim - cs)
                    out.append((src.at[pl.ds(st, sz), pl.ds(cs, n)], dst.at[pl.ds(st, sz), pl.ds(cs, n)]))
            return out

        def start_all(ps, s):
            n = len(ps)
            seg = -(-n // nsw)
            order_ = []
            for j in range(seg):
                for t in range(nsw):
                    ln = min(seg, n - t * seg)
                    if j < ln:
                        order_.append(t * seg + (j + (wshift if t % 2 else 0)) % ln)
            assert sorted(order_) == list(range(n))
            for j, idx in enumerate(order_):
                a, b_ = ps[idx]
                pltpu.make_async_copy(a, b_, s).start(priority=j % 2)

        def start_w(src, dst, s, prows, r0=0, nr=None):
            start_all(pieces(src, dst, r0, src.shape[0] if nr is None else nr, prows), s)

        def wait_buf(buf, s):
            pltpu.make_async_copy(buf, buf, s).wait()

        def start_head(hh, slot):
            for st in range(0, W, rows):
                for b in range(B):
                    for t, (src, shift) in enumerate(((k_hbm, kshift), (v_hbm, vshift))):
                        r = (st + shift + b * e) % W
                        for a_, n_ in ([(r, rows)] if r + rows <= W else [(r, W - r), (0, rows - (W - r))]):
                            pltpu.make_async_copy(src.at[b, hh, pl.ds(S - W + a_, n_), :], kv.at[slot, t, b, pl.ds(a_, n_), :], sem.at[slot]).start(priority=t)

        ws = sem.at[depth]
        cp_c = pltpu.make_async_copy(c_hbm, cb_, ws)
        cp_x = pltpu.make_async_copy(x_hbm, xb, ws)
        start_w(wm_hbm, wmb, ws, prows0)
        cp_c.start(priority=0)
        cp_x.start(priority=1)
        start_w(wq_hbm, wqb, sem.at[depth - 1], prows0)
        with scope("W_wm"):
            cp_c.wait()
            cp_x.wait()
            wait_buf(wmb, ws)
        sc = _silu(cb_[...].astype(F32)).astype(BF16)
        mod = jnp.dot(sc, wmb[...], preferred_element_type=F32)
        sa, ca, ga, sb, cb, gb = [mod[:, j * D:(j + 1) * D] for j in range(6)]
        x = xb[...].astype(F32)
        h = (_layernorm(x) * (1.0 + ca) + sa).astype(BF16)
        for i in range(depth - 1):
            start_head(i, i)
        with scope("W_wq"):
            wait_buf(wqb, sem.at[depth - 1])
        q = jnp.dot(h, wqb[...], preferred_element_type=F32)
        for hh in range(H):
            qs[hh] = q[:, hh * Dh:(hh + 1) * Dh]
        start_head(depth - 1, depth - 1)

        scale = Dh ** -0.5
        row = lax.broadcasted_iota(jnp.int32, (B, Dh), 0)

        def attend(hh):
            slot = hh % depth
            with scope("W_kv"):
                wait_buf(kv.at[slot], sem.at[slot])
            qh = qs[hh].astype(BF16)
            s0 = lax.dot_general(qh, kv[slot, 0, 0], NT, preferred_element_type=F32)
            s1 = lax.dot_general(qh, kv[slot, 0, 1], NT, preferred_element_type=F32)
            s = jnp.where(lax.broadcasted_iota(jnp.int32, s0.shape, 0) == 0, s0, s1) * scale
            m = jnp.max(s, axis=-1, keepdims=True)
            p = jnp.exp(s - m)
            l = jnp.sum(p, axis=-1, keepdims=True)
            pb = p.astype(BF16)
            o0 = jnp.dot(pb, kv[slot, 1, 0], preferred_element_type=F32)
            o1 = jnp.dot(pb, kv[slot, 1, 1], preferred_element_type=F32)
            os_[hh] = jnp.where(row == 0, o0, o1) / l

        def body(hh, _):
            attend(hh)
            start_head(hh + depth, hh % depth)
            return 0

        lax.fori_loop(0, H - depth, body, 0)
        sl = [sem.at[0], sem.at[1], sem.at[3]]

        def start_last():
            p3 = [(a_, b_, sl[1]) for a_, b_ in pieces(w3_hbm, w3b, 0, F, prows1)]
            p2 = [(a_, b_, sl[2]) for a_, b_ in pieces(w2_hbm, w2b, *w2_chunks[0], prows1)]
            for j in range(max(len(p3), len(p2))):
                if j < len(p3):
                    pltpu.make_async_copy(*p3[j]).start(priority=0)
                if j < len(p2):
                    pltpu.make_async_copy(*p2[j]).start(priority=1)

        tail = [lambda: (start_w(wo_hbm, wob, ws, prows1), start_w(w1_hbm, w1b, sl[0], prows1)),
                start_last]

        def body2(i, _):
            attend(i)
            for j in range(depth):
                @pl.when(i == H - depth + j)
                def _():
                    tail[j]()
            return 0
        lax.fori_loop(H - depth, H, body2, 0)

        with scope("W_wo"):
            wait_buf(wob, ws)
        for j, (a_, b_) in enumerate(pieces(w2_hbm, w2b, *w2_chunks[1], prows1)):
            pltpu.make_async_copy(a_, b_, ws).start(priority=lastp[j % len(lastp)])
        o_all = jnp.concatenate([os_[hh] for hh in range(H)], axis=-1)
        attn = jnp.dot(o_all.astype(BF16), wob[...], preferred_element_type=F32)
        x1 = x + ga * attn
        h2 = (_layernorm(x1) * (1.0 + cb) + sb).astype(BF16)
        with scope("W_w1"):
            wait_buf(w1b, sl[0])
        gate = lax.dot_general(h2, w1b[...], NT, preferred_element_type=F32)
        gs = _silu(gate)
        with scope("W_w3"):
            wait_buf(w3b, sl[1])
        up = lax.dot_general(h2, w3b[...], NT, preferred_element_type=F32)
        act = (gs * up).astype(BF16)
        (s0, n0), (s1, n1) = w2_chunks
        with scope("W_w2"):
            wait_buf(w2b.at[pl.ds(s0, n0), :], sl[2])
        accb[...] = x1 + gb * jnp.dot(act[:, s0:s0 + n0], w2b[pl.ds(s0, n0), :], preferred_element_type=F32)
        with scope("W_w2"):
            wait_buf(w2b.at[pl.ds(s1, n1), :], ws)
        ob[...] = (accb[...] + gb * jnp.dot(act[:, s1:s1 + n1], w2b[pl.ds(s1, n1), :], preferred_element_type=F32)).astype(BF16)
        cp_o = pltpu.make_async_copy(ob, o_hbm, sl[1])
        cp_o.start()
        with scope("W_o"):
            cp_o.wait()

    def fn(A_x, A_k_cache, A_v_cache, A_wq, A_wo, B_x, B_w1, B_w3, B_w2, c, w_mod):
        any_ = pl.BlockSpec(memory_space=pl.ANY)
        out = pl.pallas_call(
            kern,
            out_shape=jax.ShapeDtypeStruct((B, D), BF16),
            in_specs=[any_] * 10,
            out_specs=any_,
            scratch_shapes=[
                pltpu.VMEM((depth, 2, B, W, Dh), BF16),
                pltpu.VMEM((B, D), BF16), pltpu.VMEM((B, D), BF16),
                pltpu.VMEM((D, 6 * D), BF16), pltpu.VMEM((D, H * Dh), BF16), pltpu.VMEM((H * Dh, D), BF16),
                pltpu.VMEM((F, D), BF16), pltpu.VMEM((F, D), BF16), pltpu.VMEM((F, D), BF16),
                pltpu.VMEM((H, B, Dh), F32), pltpu.VMEM((H, B, Dh), F32),
                pltpu.VMEM((B, D), F32), pltpu.VMEM((B, D), BF16), pltpu.SemaphoreType.DMA((4,)),
            ],
            compiler_params=pltpu.CompilerParams(vmem_limit_bytes=100 * 1024 * 1024, disable_bounds_checks=nochk, disable_semaphore_checks=nochk),
            name=name,
        )(A_x.reshape(B, D), A_k_cache, A_v_cache, A_wq, A_wo, B_w1.T, B_w3.T, B_w2, c, w_mod)
        return out.reshape(B, 1, D)
    return fn


_kernel = make("adaln_decode", )


@jax.jit
def pallas_adaLN_cond__sliding_block_cached__glu_gated_swiglu__decode_kernel(
    A_x, A_k_cache, A_v_cache, A_wq, A_wo, B_x, B_w1, B_w3, B_w2, c, w_mod):
    return _kernel(A_x, A_k_cache, A_v_cache, A_wq, A_wo, B_x, B_w1, B_w3, B_w2, c, w_mod)
```

```python
import contextlib
import jax
import jax.numpy as jnp
from jax import lax
import jax.experimental.pallas as pl
import jax.experimental.pallas.tpu as pltpu

F32 = jnp.float32
BF16 = jnp.bfloat16
NT = (((1,), (1,)), ((), ()))


def _silu(x):
    return x * (1.0 / (1.0 + jnp.exp(-x)))


def _layernorm(x, eps=1e-5):
    m = jnp.mean(x, axis=-1, keepdims=True)
    d = x - m
    v = jnp.mean(d * d, axis=-1, keepdims=True)
    return d / jnp.sqrt(v + eps)


def make(name="k7", rows=128, kshift=0, vshift=64, nsw=8, wshift=5, nparts=4, scopes=False, nochk=True,
         w2_chunks=((0, 1024), (1024, 352)), lastp=(1,)):
    B, H, S, Dh, D, F = 2, 32, 16384, 128, 512, 1376
    W = min(4096, max(256, S // 4))
    G = 8
    NG = B * H // G
    GPB = H // G
    piece = rows * Dh
    scope = (lambda n: jax.named_scope(n)) if scopes else (lambda n: contextlib.nullcontext())

    def kern(x_hbm, k_hbm, v_hbm, wq_hbm, wo_hbm, w1_hbm, w3_hbm, w2_hbm, c_hbm, wm_hbm, o_hbm,
             kb, vb, xb, cb_, wmb, wqb, wob, w1b, w3b, w2b, qs, os_, accb, ob, sem):

        def pieces(src, dst, r0, nr):
            cdim = src.shape[1]
            lanes = min(cdim, piece // 8)
            step = piece // lanes
            out = []
            for st in range(r0, r0 + nr, step):
                sz = min(step, r0 + nr - st)
                for cs in range(0, cdim, lanes):
                    n = min(lanes, cdim - cs)
                    out.append((src.at[pl.ds(st, sz), pl.ds(cs, n)], dst.at[pl.ds(st, sz), pl.ds(cs, n)]))
            return out

        def start_w(src, dst, s):
            ps = pieces(src, dst, 0, src.shape[0])
            n = len(ps)
            seg = -(-n // nsw)
            order = []
            for j in range(seg):
                for t in range(nsw):
                    ln = min(seg, n - t * seg)
                    if j < ln:
                        order.append(t * seg + (j + (wshift if t % 2 else 0)) % ln)
            assert sorted(order) == list(range(n))
            for j, idx in enumerate(order):
                pltpu.make_async_copy(*ps[idx], s).start(priority=j % 2)

        def wait_buf(buf, s):
            pltpu.make_async_copy(buf, buf, s).wait()

        def start_group(src, dst, shift, g, s, part=0, nparts=1):
            b = g // GPB
            h0 = (g % GPB) * G
            n = W // nparts
            for st in range(part * n, (part + 1) * n, rows):
                r = (st + shift) % W
                for j in range(G):
                    for a, ln in ([(r, rows)] if r + rows <= W else [(r, W - r), (0, rows - (W - r))]):
                        pltpu.make_async_copy(src.at[b, h0 + j, pl.ds(S - W + a, ln), :],
                                              dst.at[j, pl.ds(a, ln), :], s).start(priority=j % 2)

        def start_k(g, **kw):
            start_group(k_hbm, kb.at[g % 2], kshift, g, sem.at[g % 2], **kw)

        def start_v(g, **kw):
            start_group(v_hbm, vb.at[g % 2], vshift, g, sem.at[2 + g % 2], **kw)

        cp_c = pltpu.make_async_copy(c_hbm, cb_, sem.at[1])
        cp_x = pltpu.make_async_copy(x_hbm, xb, sem.at[1])
        start_w(wm_hbm, wmb, sem.at[1])
        cp_c.start(priority=0)
        cp_x.start(priority=1)
        start_w(wq_hbm, wqb, sem.at[3])
        with scope("W_wm"):
            cp_c.wait()
            cp_x.wait()
            wait_buf(wmb, sem.at[1])
        start_k(0, part=0, nparts=4)
        sc = _silu(cb_[...].astype(F32)).astype(BF16)
        mod = jnp.dot(sc, wmb[...], preferred_element_type=F32)
        sa, ca, ga, sb, cb, gb = [mod[:, j * D:(j + 1) * D] for j in range(6)]
        x = xb[...].astype(F32)
        h = (_layernorm(x) * (1.0 + ca) + sa).astype(BF16)
        start_k(0, part=1, nparts=4)
        with scope("W_wq"):
            wait_buf(wqb, sem.at[3])
        q = jnp.dot(h, wqb[...], preferred_element_type=F32)
        for hh in range(H):
            for b in range(B):
                qs[b * GPB + hh // G, pl.ds(hh % G, 1), :] = q[b:b + 1, hh * Dh:(hh + 1) * Dh]
        start_k(0, part=2, nparts=4)
        start_k(0, part=3, nparts=4)
        start_v(0)

        scale = Dh ** -0.5
        per = G // nparts

        def attend(g, issue_a, issue_b):
            slot = g % 2
            with scope("W_k"):
                wait_buf(kb.at[slot], sem.at[slot])
            qg = qs[g].astype(BF16)
            srow = lax.broadcasted_iota(jnp.int32, (G, W), 0)
            s = None
            for j in range(G):
                sj = lax.dot_general(qg, kb[slot, j], NT, preferred_element_type=F32)
                s = sj if s is None else jnp.where(srow == j, sj, s)
                if (j + 1) % per == 0:
                    issue_a(j // per)
            s = s * scale
            m = jnp.max(s, axis=-1, keepdims=True)
            p = jnp.exp(s - m)
            l = jnp.sum(p, axis=-1, keepdims=True)
            pb = p.astype(BF16)
            with scope("W_v"):
                wait_buf(vb.at[slot], sem.at[2 + slot])
            orow = lax.broadcasted_iota(jnp.int32, (G, Dh), 0)
            o = None
            for j in range(G):
                oj = jnp.dot(pb, vb[slot, j], preferred_element_type=F32)
                o = oj if o is None else jnp.where(orow == j, oj, o)
                if (j + 1) % per == 0:
                    issue_b(j // per)
            os_[g] = o / l

        def body(g, _):
            attend(g, lambda part: start_k(g + 1, part=part, nparts=nparts),
                   lambda part: start_v(g + 1, part=part, nparts=nparts))
            return 0

        lax.fori_loop(0, NG - 1, body, 0)

        def issue_a(part):
            if part == 0:
                start_w(wo_hbm, wob, sem.at[0])
            if part == nparts - 1:
                start_w(w1_hbm, w1b, sem.at[2])

        def issue_b(part):
            if part == nparts // 2 - 1:
                p3 = pieces(w3_hbm, w3b, 0, F)
                p2 = pieces(w2_hbm, w2b, *w2_chunks[0])
                for j in range(max(len(p3), len(p2))):
                    if j < len(p3):
                        pltpu.make_async_copy(*p3[j], sem.at[1]).start(priority=0)
                    if j < len(p2):
                        pltpu.make_async_copy(*p2[j], sem.at[3]).start(priority=1)

        attend(NG - 1, issue_a, issue_b)

        with scope("W_wo"):
            wait_buf(wob, sem.at[0])
        for j, pc in enumerate(pieces(w2_hbm, w2b, *w2_chunks[1])):
            pltpu.make_async_copy(*pc, sem.at[0]).start(priority=lastp[j % len(lastp)])
        o_all = jnp.concatenate(
            [jnp.concatenate([os_[b * GPB + hh // G, pl.ds(hh % G, 1), :] for b in range(B)], axis=0)
             for hh in range(H)], axis=-1)
        attn = jnp.dot(o_all.astype(BF16), wob[...], preferred_element_type=F32)
        x1 = x + ga * attn
        h2 = (_layernorm(x1) * (1.0 + cb) + sb).astype(BF16)
        with scope("W_w1"):
            wait_buf(w1b, sem.at[2])
        gate = lax.dot_general(h2, w1b[...], NT, preferred_element_type=F32)
        gs = _silu(gate)
        with scope("W_w3"):
            wait_buf(w3b, sem.at[1])
        up = lax.dot_general(h2, w3b[...], NT, preferred_element_type=F32)
        act = (gs * up).astype(BF16)
        (s0, n0), (s1, n1) = w2_chunks
        with scope("W_w2"):
            wait_buf(w2b.at[pl.ds(s0, n0), :], sem.at[3])
        accb[...] = x1 + gb * jnp.dot(act[:, s0:s0 + n0], w2b[pl.ds(s0, n0), :], preferred_element_type=F32)
        with scope("W_w2"):
            wait_buf(w2b.at[pl.ds(s1, n1), :], sem.at[0])
        ob[...] = (accb[...] + gb * jnp.dot(act[:, s1:s1 + n1], w2b[pl.ds(s1, n1), :],
                                            preferred_element_type=F32)).astype(BF16)
        cp_o = pltpu.make_async_copy(ob, o_hbm, sem.at[1])
        cp_o.start()
        with scope("W_o"):
            cp_o.wait()

    def fn(A_x, A_k_cache, A_v_cache, A_wq, A_wo, B_x, B_w1, B_w3, B_w2, c, w_mod):
        any_ = pl.BlockSpec(memory_space=pl.ANY)
        out = pl.pallas_call(
            kern,
            out_shape=jax.ShapeDtypeStruct((B, D), BF16),
            in_specs=[any_] * 10,
            out_specs=any_,
            scratch_shapes=[
                pltpu.VMEM((2, G, W, Dh), BF16), pltpu.VMEM((2, G, W, Dh), BF16),
                pltpu.VMEM((B, D), BF16), pltpu.VMEM((B, D), BF16),
                pltpu.VMEM((D, 6 * D), BF16), pltpu.VMEM((D, H * Dh), BF16), pltpu.VMEM((H * Dh, D), BF16),
                pltpu.VMEM((F, D), BF16), pltpu.VMEM((F, D), BF16), pltpu.VMEM((F, D), BF16),
                pltpu.VMEM((NG, G, Dh), F32), pltpu.VMEM((NG, G, Dh), F32),
                pltpu.VMEM((B, D), F32), pltpu.VMEM((B, D), BF16), pltpu.SemaphoreType.DMA((4,)),
            ],
            compiler_params=pltpu.CompilerParams(vmem_limit_bytes=100 * 1024 * 1024,
                                                 disable_bounds_checks=nochk, disable_semaphore_checks=nochk),
            name=name,
        )(A_x.reshape(B, D), A_k_cache, A_v_cache, A_wq, A_wo, B_w1.T, B_w3.T, B_w2, c, w_mod)
        return out.reshape(B, 1, D)
    return fn


_kernel = make("adaln_decode", )


@jax.jit
def pallas_adaLN_cond__sliding_block_cached__glu_gated_swiglu__decode_kernel(
    A_x, A_k_cache, A_v_cache, A_wq, A_wo, B_x, B_w1, B_w3, B_w2, c, w_mod):
    return _kernel(A_x, A_k_cache, A_v_cache, A_wq, A_wo, B_x, B_w1, B_w3, B_w2, c, w_mod)
```

```python
import jax
import jax.numpy as jnp
from jax import lax
import jax.experimental.pallas as pl
import jax.experimental.pallas.tpu as pltpu

F32 = jnp.float32
BF16 = jnp.bfloat16
NT = (((1,), (1,)), ((), ()))

HQ, DH = 32, 128
G = 8
ROWS = 128
PIECE = ROWS * DH
V_SHIFT = 64
W_STREAMS = 8
W_SHIFT = 5
PARTS = 4
W2_TAIL = 224


def _silu(x):
    return x * lax.logistic(x)


def _layernorm(x, eps=1e-5):
    m = jnp.mean(x, axis=-1, keepdims=True)
    d = x - m
    v = jnp.mean(d * d, axis=-1, keepdims=True)
    return d / jnp.sqrt(v + eps)


def _pieces(src, dst, r0, nr):
    cols = src.shape[1]
    lanes = min(cols, PIECE // 8)
    step = PIECE // lanes
    out = []
    for r in range(r0, r0 + nr, step):
        rn = min(step, r0 + nr - r)
        for c in range(0, cols, lanes):
            cn = min(lanes, cols - c)
            out.append((src.at[pl.ds(r, rn), pl.ds(c, cn)],
                        dst.at[pl.ds(r, rn), pl.ds(c, cn)]))
    return out


def _start_weight(src, dst, sem):
    ps = _pieces(src, dst, 0, src.shape[0])
    n = len(ps)
    seg = -(-n // W_STREAMS)
    order = []
    for j in range(seg):
        for t in range(W_STREAMS):
            ln = min(seg, n - t * seg)
            if j < ln:
                order.append(t * seg + (j + (W_SHIFT if t % 2 else 0)) % ln)
    assert sorted(order) == list(range(n))
    for j, idx in enumerate(order):
        pltpu.make_async_copy(*ps[idx], sem).start(priority=j % 2)


def _wait_filled(buf, sem):
    pltpu.make_async_copy(buf, buf, sem).wait()


def _kernel(x_hbm, k_hbm, v_hbm, wq_hbm, wo_hbm, w1t_hbm, w3t_hbm, w2_hbm, c_hbm, wm_hbm,
            o_hbm,
            kb, vb, xb, cb_in, wmb, wqb, wob, w1b, w3b, w2b, qs, ao, accb, ob, sem):
    B, D = x_hbm.shape
    S = k_hbm.shape[2]
    W = kb.shape[2]
    F = w2_hbm.shape[0]
    gpb = HQ // G
    ng = B * gpb
    dots_per_part = G // PARTS

    def start_group(src, dst, shift, g, s, part, parts):
        b = g // gpb
        h0 = (g % gpb) * G
        n = W // parts
        for st in range(part * n, (part + 1) * n, ROWS):
            r = (st + shift) % W
            spans = [(r, ROWS)] if r + ROWS <= W else [(r, W - r), (0, r + ROWS - W)]
            for j in range(G):
                for a, ln in spans:
                    pltpu.make_async_copy(
                        src.at[b, h0 + j, pl.ds(S - W + a, ln), :],
                        dst.at[j, pl.ds(a, ln), :], s).start(priority=j % 2)

    def start_k(g, part=0, parts=PARTS):
        start_group(k_hbm, kb.at[g % 2], 0, g, sem.at[g % 2], part, parts)

    def start_v(g, part=0, parts=PARTS):
        start_group(v_hbm, vb.at[g % 2], V_SHIFT, g, sem.at[2 + g % 2], part, parts)

    cp_c = pltpu.make_async_copy(c_hbm, cb_in, sem.at[1])
    cp_x = pltpu.make_async_copy(x_hbm, xb, sem.at[1])
    _start_weight(wm_hbm, wmb, sem.at[1])
    cp_c.start(priority=0)
    cp_x.start(priority=1)
    _start_weight(wq_hbm, wqb, sem.at[3])
    cp_c.wait()
    cp_x.wait()
    _wait_filled(wmb, sem.at[1])
    start_k(0, 0, 4)
    mod = jnp.dot(_silu(cb_in[...].astype(F32)).astype(BF16), wmb[...],
                  preferred_element_type=F32)
    sa, ca, ga, sb, cb, gb = [mod[:, j * D:(j + 1) * D] for j in range(6)]
    x = xb[...].astype(F32)
    h = (_layernorm(x) * (1.0 + ca) + sa).astype(BF16)
    start_k(0, 1, 4)
    _wait_filled(wqb, sem.at[3])
    q = jnp.dot(h, wqb[...], preferred_element_type=F32)
    for hh in range(HQ):
        for b in range(B):
            qs[b * gpb + hh // G, pl.ds(hh % G, 1), :] = q[b:b + 1, hh * DH:(hh + 1) * DH]
    start_k(0, 2, 4)
    start_k(0, 3, 4)
    start_v(0, 0, 1)

    def attend(g, issue_during_qk, issue_during_pv):
        slot = g % 2
        _wait_filled(kb.at[slot], sem.at[slot])
        qg = qs[g].astype(BF16)
        srow = lax.broadcasted_iota(jnp.int32, (G, W), 0)
        s = None
        for j in range(G):
            sj = lax.dot_general(qg, kb[slot, j], NT, preferred_element_type=F32)
            s = sj if s is None else jnp.where(srow == j, sj, s)
            if (j + 1) % dots_per_part == 0:
                issue_during_qk(j // dots_per_part)
        s = s * (DH ** -0.5)
        m = jnp.max(s, axis=-1, keepdims=True)
        p = jnp.exp(s - m)
        l = jnp.sum(p, axis=-1, keepdims=True)
        pb = p.astype(BF16)
        _wait_filled(vb.at[slot], sem.at[2 + slot])
        orow = lax.broadcasted_iota(jnp.int32, (G, DH), 0)
        o = None
        for j in range(G):
            oj = jnp.dot(pb, vb[slot, j], preferred_element_type=F32)
            o = oj if o is None else jnp.where(orow == j, oj, o)
            if (j + 1) % dots_per_part == 0:
                issue_during_pv(j // dots_per_part)
        ao[g] = o / l

    def body(g, carry):
        attend(g, lambda part: start_k(g + 1, part), lambda part: start_v(g + 1, part))
        return carry

    lax.fori_loop(0, ng - 1, body, 0)

    last = (ng - 1) % 2
    sem_wo, sem_w1 = sem.at[1 - last], sem.at[3 - last]
    sem_w3, sem_w2 = sem.at[last], sem.at[2 + last]
    f0 = F - W2_TAIL

    def issue_wo_w1(part):
        if part == 0:
            _start_weight(wo_hbm, wob, sem_wo)
        if part == PARTS - 1:
            _start_weight(w1t_hbm, w1b, sem_w1)

    def issue_w3_w2(part):
        if part == PARTS // 2 - 1:
            p3 = _pieces(w3t_hbm, w3b, 0, F)
            p2 = _pieces(w2_hbm, w2b, 0, f0)
            for j in range(max(len(p3), len(p2))):
                if j < len(p3):
                    pltpu.make_async_copy(*p3[j], sem_w3).start(priority=0)
                if j < len(p2):
                    pltpu.make_async_copy(*p2[j], sem_w2).start(priority=1)

    attend(ng - 1, issue_wo_w1, issue_w3_w2)

    _wait_filled(wob, sem_wo)
    for pc in _pieces(w2_hbm, w2b, f0, W2_TAIL):
        pltpu.make_async_copy(*pc, sem_wo).start(priority=1)
    o_all = jnp.concatenate(
        [jnp.concatenate([ao[b * gpb + hh // G, pl.ds(hh % G, 1), :] for b in range(B)], axis=0)
         for hh in range(HQ)], axis=-1)
    x1 = x + ga * jnp.dot(o_all.astype(BF16), wob[...], preferred_element_type=F32)
    h2 = (_layernorm(x1) * (1.0 + cb) + sb).astype(BF16)
    _wait_filled(w1b, sem_w1)
    gate = _silu(lax.dot_general(h2, w1b[...], NT, preferred_element_type=F32))
    _wait_filled(w3b, sem_w3)
    up = lax.dot_general(h2, w3b[...], NT, preferred_element_type=F32)
    act = (gate * up).astype(BF16)
    _wait_filled(w2b.at[pl.ds(0, f0), :], sem_w2)
    accb[...] = x1 + gb * jnp.dot(act[:, :f0], w2b[pl.ds(0, f0), :],
                                  preferred_element_type=F32)
    _wait_filled(w2b.at[pl.ds(f0, W2_TAIL), :], sem_wo)
    ob[...] = (accb[...] + gb * jnp.dot(act[:, f0:], w2b[pl.ds(f0, W2_TAIL), :],
                                        preferred_element_type=F32)).astype(ob.dtype)
    cp_o = pltpu.make_async_copy(ob, o_hbm, sem_w3)
    cp_o.start()
    cp_o.wait()


@jax.jit
def pallas_adaLN_cond__sliding_block_cached__glu_gated_swiglu__decode_kernel(
    A_x: jax.Array,
    A_k_cache: jax.Array,
    A_v_cache: jax.Array,
    A_wq: jax.Array,
    A_wo: jax.Array,
    B_x: jax.Array,
    B_w1: jax.Array,
    B_w3: jax.Array,
    B_w2: jax.Array,
    c: jax.Array,
    w_mod: jax.Array,
):
    del B_x
    B, Sq, D = A_x.shape
    _, Hkv, Sk, Dh = A_k_cache.shape
    F = B_w2.shape[0]
    W = min(4096, max(256, Sk // 4))
    assert Sq == 1 and Hkv == HQ and Dh == DH and W % (4 * ROWS) == 0
    ng = B * HQ // G
    dt = A_x.dtype

    hbm = pl.BlockSpec(memory_space=pl.ANY)
    out = pl.pallas_call(
        _kernel,
        out_shape=jax.ShapeDtypeStruct((B, D), dt),
        in_specs=[hbm] * 10,
        out_specs=hbm,
        scratch_shapes=[
            pltpu.VMEM((2, G, W, DH), dt),
            pltpu.VMEM((2, G, W, DH), dt),
            pltpu.VMEM((B, D), dt),
            pltpu.VMEM((B, D), dt),
            pltpu.VMEM(w_mod.shape, dt),
            pltpu.VMEM(A_wq.shape, dt),
            pltpu.VMEM(A_wo.shape, dt),
            pltpu.VMEM((F, D), dt),
            pltpu.VMEM((F, D), dt),
            pltpu.VMEM((F, D), dt),
            pltpu.VMEM((ng, G, DH), F32),
            pltpu.VMEM((ng, G, DH), F32),
            pltpu.VMEM((B, D), F32),
            pltpu.VMEM((B, D), dt),
            pltpu.SemaphoreType.DMA((4,)),
        ],
        compiler_params=pltpu.CompilerParams(vmem_limit_bytes=100 * 1024 * 1024),
        name="adaln_swa_swiglu_decode",
    )(A_x.reshape(B, D), A_k_cache, A_v_cache, A_wq, A_wo, B_w1.T, B_w3.T, B_w2, c, w_mod)
    return out.reshape(B, Sq, D)
```

```python
import jax
import jax.numpy as jnp
from jax import lax
import jax.experimental.pallas as pl
import jax.experimental.pallas.tpu as pltpu

F32 = jnp.float32
BF16 = jnp.bfloat16
NT = (((1,), (1,)), ((), ()))

HQ, DH = 32, 128
G = 8
ROWS = 128
PIECE = ROWS * DH
V_SHIFT = 64
W_STREAMS = 8
W_SHIFT = 5
PARTS = 4
W2_TAIL = 224


def _silu(x):
    return x * lax.logistic(x)


def _layernorm(x, eps=1e-5):
    m = jnp.mean(x, axis=-1, keepdims=True)
    d = x - m
    v = jnp.mean(d * d, axis=-1, keepdims=True)
    return d / jnp.sqrt(v + eps)


def _pieces(src, dst, r0, nr):
    cols = src.shape[1]
    lanes = min(cols, PIECE // 8)
    step = PIECE // lanes
    out = []
    for r in range(r0, r0 + nr, step):
        rn = min(step, r0 + nr - r)
        for c in range(0, cols, lanes):
            cn = min(lanes, cols - c)
            out.append((src.at[pl.ds(r, rn), pl.ds(c, cn)],
                        dst.at[pl.ds(r, rn), pl.ds(c, cn)]))
    return out


def _start_weight(src, dst, sem):
    ps = _pieces(src, dst, 0, src.shape[0])
    n = len(ps)
    seg = -(-n // W_STREAMS)
    order = []
    for j in range(seg):
        for t in range(W_STREAMS):
            ln = min(seg, n - t * seg)
            if j < ln:
                order.append(t * seg + (j + (W_SHIFT if t % 2 else 0)) % ln)
    assert sorted(order) == list(range(n))
    for j, idx in enumerate(order):
        pltpu.make_async_copy(*ps[idx], sem).start(priority=j % 2)


def _wait_filled(buf, sem):
    pltpu.make_async_copy(buf, buf, sem).wait()


def _kernel(x_hbm, k_hbm, v_hbm, wq_hbm, wo_hbm, w1t_hbm, w3t_hbm, w2_hbm, c_hbm, wm_hbm,
            o_hbm,
            kb, vb, xb, cb_in, wmb, wqb, wob, w1b, w3b, w2b, qs, ao, accb, ob, sem):
    B, D = x_hbm.shape
    S = k_hbm.shape[2]
    W = kb.shape[2]
    F = w2_hbm.shape[0]
    gpb = HQ // G
    ng = B * gpb
    dots_per_part = G // PARTS

    def place(b, hh):
        return b * gpb + hh // (2 * G) * 2 + hh % 2, hh % (2 * G) // 2

    def start_group(src, dst, shift, g, s, part, parts):
        b = g // gpb
        h0 = (g % gpb) // 2 * (2 * G) + g % 2
        n = W // parts
        for st in range(part * n, (part + 1) * n, ROWS):
            r = (st + shift) % W
            spans = [(r, ROWS)] if r + ROWS <= W else [(r, W - r), (0, r + ROWS - W)]
            for j in range(G):
                for a, ln in spans:
                    pltpu.make_async_copy(
                        src.at[b, h0 + 2 * j, pl.ds(S - W + a, ln), :],
                        dst.at[j, pl.ds(a, ln), :], s).start(priority=j % 2)

    def start_k(g, part=0, parts=PARTS):
        start_group(k_hbm, kb.at[g % 2], 0, g, sem.at[g % 2], part, parts)

    def start_v(g, part=0, parts=PARTS):
        start_group(v_hbm, vb.at[g % 2], V_SHIFT, g, sem.at[2 + g % 2], part, parts)

    cp_c = pltpu.make_async_copy(c_hbm, cb_in, sem.at[2])
    cp_x = pltpu.make_async_copy(x_hbm, xb, sem.at[2])
    _start_weight(wm_hbm, wmb, sem.at[1])
    cp_c.start(priority=0)
    cp_x.start(priority=1)
    _start_weight(wq_hbm, wqb, sem.at[3])
    cp_c.wait()
    cp_x.wait()
    _wait_filled(wmb, sem.at[1])
    start_k(0, 0, 4)
    mod = jnp.dot(_silu(cb_in[...].astype(F32)).astype(BF16), wmb[...],
                  preferred_element_type=F32)
    sa, ca, ga, sb, cb, gb = [mod[:, j * D:(j + 1) * D] for j in range(6)]
    x = xb[...].astype(F32)
    h = (_layernorm(x) * (1.0 + ca) + sa).astype(BF16)
    start_k(0, 1, 4)
    _wait_filled(wqb, sem.at[3])
    q = jnp.dot(h, wqb[...], preferred_element_type=F32)
    for hh in range(HQ):
        for b in range(B):
            g, row = place(b, hh)
            qs[g, pl.ds(row, 1), :] = q[b:b + 1, hh * DH:(hh + 1) * DH]
    start_k(0, 2, 4)
    start_k(0, 3, 4)
    start_v(0, 0, 1)

    def attend(g, issue_during_qk, issue_during_pv):
        slot = g % 2
        _wait_filled(kb.at[slot], sem.at[slot])
        qg = qs[g].astype(BF16)
        srow = lax.broadcasted_iota(jnp.int32, (G, W), 0)
        s = None
        for j in range(G):
            sj = lax.dot_general(qg, kb[slot, j], NT, preferred_element_type=F32)
            s = sj if s is None else jnp.where(srow == j, sj, s)
            if (j + 1) % dots_per_part == 0:
                issue_during_qk(j // dots_per_part)
        s = s * (DH ** -0.5)
        m = jnp.max(s, axis=-1, keepdims=True)
        p = jnp.exp(s - m)
        l = jnp.sum(p, axis=-1, keepdims=True)
        pb = p.astype(BF16)
        _wait_filled(vb.at[slot], sem.at[2 + slot])
        orow = lax.broadcasted_iota(jnp.int32, (G, DH), 0)
        o = None
        for j in range(G):
            oj = jnp.dot(pb, vb[slot, j], preferred_element_type=F32)
            o = oj if o is None else jnp.where(orow == j, oj, o)
            if (j + 1) % dots_per_part == 0:
                issue_during_pv(j // dots_per_part)
        ao[g] = o / l

    def body(g, carry):
        attend(g, lambda part: start_k(g + 1, part), lambda part: start_v(g + 1, part))
        return carry

    lax.fori_loop(0, ng - 1, body, 0)

    last = (ng - 1) % 2
    sem_wo, sem_w1 = sem.at[1 - last], sem.at[3 - last]
    sem_w3, sem_w2 = sem.at[last], sem.at[2 + last]
    f0 = F - W2_TAIL

    def issue_wo_w1(part):
        if part == 0:
            _start_weight(wo_hbm, wob, sem_wo)
        if part == PARTS - 1:
            _start_weight(w1t_hbm, w1b, sem_w1)

    def issue_w3_w2(part):
        if part == PARTS // 2 - 1:
            p3 = _pieces(w3t_hbm, w3b, 0, F)
            p2 = _pieces(w2_hbm, w2b, 0, f0)
            for j in range(max(len(p3), len(p2))):
                if j < len(p3):
                    pltpu.make_async_copy(*p3[j], sem_w3).start(priority=0)
                if j < len(p2):
                    pltpu.make_async_copy(*p2[j], sem_w2).start(priority=1)

    attend(ng - 1, issue_wo_w1, issue_w3_w2)

    _wait_filled(wob, sem_wo)
    for pc in _pieces(w2_hbm, w2b, f0, W2_TAIL):
        pltpu.make_async_copy(*pc, sem_wo).start(priority=1)
    o_all = jnp.concatenate(
        [jnp.concatenate([ao[place(b, hh)[0], pl.ds(place(b, hh)[1], 1), :] for b in range(B)],
                         axis=0)
         for hh in range(HQ)], axis=-1)
    x1 = x + ga * jnp.dot(o_all.astype(BF16), wob[...], preferred_element_type=F32)
    h2 = (_layernorm(x1) * (1.0 + cb) + sb).astype(BF16)
    _wait_filled(w1b, sem_w1)
    gate = _silu(lax.dot_general(h2, w1b[...], NT, preferred_element_type=F32))
    _wait_filled(w3b, sem_w3)
    up = lax.dot_general(h2, w3b[...], NT, preferred_element_type=F32)
    act = (gate * up).astype(BF16)
    _wait_filled(w2b.at[pl.ds(0, f0), :], sem_w2)
    accb[...] = x1 + gb * jnp.dot(act[:, :f0], w2b[pl.ds(0, f0), :],
                                  preferred_element_type=F32)
    _wait_filled(w2b.at[pl.ds(f0, W2_TAIL), :], sem_wo)
    ob[...] = (accb[...] + gb * jnp.dot(act[:, f0:], w2b[pl.ds(f0, W2_TAIL), :],
                                        preferred_element_type=F32)).astype(ob.dtype)
    cp_o = pltpu.make_async_copy(ob, o_hbm, sem_w3)
    cp_o.start()
    cp_o.wait()


@jax.jit
def pallas_adaLN_cond__sliding_block_cached__glu_gated_swiglu__decode_kernel(
    A_x: jax.Array,
    A_k_cache: jax.Array,
    A_v_cache: jax.Array,
    A_wq: jax.Array,
    A_wo: jax.Array,
    B_x: jax.Array,
    B_w1: jax.Array,
    B_w3: jax.Array,
    B_w2: jax.Array,
    c: jax.Array,
    w_mod: jax.Array,
):
    del B_x
    B, Sq, D = A_x.shape
    _, Hkv, Sk, Dh = A_k_cache.shape
    F = B_w2.shape[0]
    W = min(4096, max(256, Sk // 4))
    assert Sq == 1 and Hkv == HQ and Dh == DH and W % (4 * ROWS) == 0
    ng = B * HQ // G
    dt = A_x.dtype

    hbm = pl.BlockSpec(memory_space=pl.ANY)
    out = pl.pallas_call(
        _kernel,
        out_shape=jax.ShapeDtypeStruct((B, D), dt),
        in_specs=[hbm] * 10,
        out_specs=hbm,
        scratch_shapes=[
            pltpu.VMEM((2, G, W, DH), dt),
            pltpu.VMEM((2, G, W, DH), dt),
            pltpu.VMEM((B, D), dt),
            pltpu.VMEM((B, D), dt),
            pltpu.VMEM(w_mod.shape, dt),
            pltpu.VMEM(A_wq.shape, dt),
            pltpu.VMEM(A_wo.shape, dt),
            pltpu.VMEM((F, D), dt),
            pltpu.VMEM((F, D), dt),
            pltpu.VMEM((F, D), dt),
            pltpu.VMEM((ng, G, DH), F32),
            pltpu.VMEM((ng, G, DH), F32),
            pltpu.VMEM((B, D), F32),
            pltpu.VMEM((B, D), dt),
            pltpu.SemaphoreType.DMA((4,)),
        ],
        compiler_params=pltpu.CompilerParams(vmem_limit_bytes=100 * 1024 * 1024),
        name="adaln_swa_swiglu_decode",
    )(A_x.reshape(B, D), A_k_cache, A_v_cache, A_wq, A_wo, B_w1.T, B_w3.T, B_w2, c, w_mod)
    return out.reshape(B, Sq, D)
```
